```python
import jax
import jax.numpy as jnp

def _softmax(x, axis=-1):
    return jax.nn.softmax(x, axis=axis)
def _gelu(x):
    return jax.nn.gelu(x, approximate=True)
def _silu(x):
    return jax.nn.silu(x)
def _sigmoid(x):
    return jax.nn.sigmoid(x)
def _layernorm(x, axis=-1, eps=1e-5):
    m = jnp.mean(x, axis=axis, keepdims=True)
    v = jnp.var(x, axis=axis, keepdims=True)
    return (x - m) / jnp.sqrt(v + eps)
def _scatter_add(tgt, idx, src, axis=0):
    return tgt.at[idx].add(src)
def _segment_sum(src, seg, n):
    return jax.ops.segment_sum(src, seg, n)
class _Rng:
    def __init__(self, key):
        self._k = key
    def _next(self):
        self._k, sub = jax.random.split(self._k)
        return sub
    def normal(self, shape):
        return jax.random.normal(self._next(), shape, dtype=jnp.bfloat16)
    def randint(self, lo, hi, shape):
        return jax.random.randint(self._next(), shape, lo, hi, dtype=jnp.int32)
    def uniform(self, shape, lo=0.0, hi=1.0):
        return jax.random.uniform(self._next(), shape, jnp.bfloat16, lo, hi)
    def permutation(self, n):
        return jax.random.permutation(self._next(), n)


kernel_name = 'standalone__mha_softmax__near_ridge'

def _fwd_setup_inputs():
    _rng = _Rng(jax.random.key(int.from_bytes(__import__("os").urandom(4), "little")))
    _w = (lambda a: (lambda t: t.astype(jnp.bfloat16) if jnp.issubdtype(t.dtype, jnp.floating) else t)(jnp.asarray(a)))
    B, H, Sq, Sk, D = 8, 16, 512, 1024, 256
    return {
        "q": _w((lambda *s: _rng.normal(s) * 0.05)(B, H, Sq, D)),
        "k": _w((lambda *s: _rng.normal(s) * 0.05)(B, H, Sk, D)),
        "v": _w((lambda *s: _rng.normal(s) * 0.05)(B, H, Sk, D)),
    }

def _fwd_reference(q, k, v):
    scale = q.shape[-1] ** -0.5
    scores = jnp.einsum("bhqd,bhkd->bhqk", q, k) * scale
    p = _softmax(scores, axis=-1)
    return jnp.einsum("bhqk,bhkd->bhqd", p, v)


def setup_inputs():
    _inp = _fwd_setup_inputs()
    _gk = jax.random.fold_in(jax.random.key(int.from_bytes(__import__("os").urandom(4), "little")), 2**31 - 1)
    _shapes = [[8, 16, 512, 256]]
    _dtypes = ['bfloat16']
    _gks = jax.random.split(_gk, len(_shapes))
    _gs = [jax.random.normal(k, s, dtype=jnp.dtype(d)) * 0.05 for k, s, d in zip(_gks, _shapes, _dtypes)]
    _inp["grad_out"] = _gs[0]
    return _inp

def reference(q, k, v, grad_out):
    _const = dict()
    def _f(*_d):
        return _fwd_reference(**{'q': _d[0], 'k': _d[1], 'v': _d[2], **_const})
    _out, _vjp = jax.vjp(_f, q, k, v)
    _grads = _vjp(grad_out)
    _out0 = jnp.asarray(_out)
    return (_out0, *[jnp.asarray(_g) for _g in _grads])
```

```python
import jax, jax.numpy as jnp
import jax.experimental.pallas as pl
import jax.experimental.pallas.tpu as pltpu

NT = (((1,), (1,)), ((), ()))
NN = (((1,), (0,)), ((), ()))
f32 = jnp.float32; bf = jnp.bfloat16
Sq, Sk, D = 512, 1024, 256
hq, hk, hd = Sq // 2, Sk // 2, D // 2
AR = ["a", "b", "11", "22", "c", "d", "e"]
BR = ["a", "11", "e", "d", "22", "c", "b"]
NAMES = ["a", "b", "c", "d", "e", "11", "22"]
HPS = 2
SCALE = D ** -0.5
C2 = SCALE * 1.4426950408889634
TN_ORDER = (2, 4, 3, 5, 1, 6, 7)

def tdot(tag, a, b, dn):
    return jax.lax.dot_general(a, b, dn, preferred_element_type=jnp.float32)

def sset(x11, x12, x21, x22):
    return {"a": x11 + x22, "b": x21 + x22, "c": x11 + x12, "d": x21 - x11, "e": x12 - x22, "11": x11, "22": x22}
def tset(x11, x12, x21, x22):
    return {"a": x11 + x22, "b": x12 + x22, "c": x11 + x21, "d": x12 - x11, "e": x21 - x22, "11": x11, "22": x22}

class Sched:
    def __init__(self):
        self.t = 0
        self.tasks = []
        self.seq = 0
    def at(self, t, fn):
        self.tasks.append((t, self.seq, fn)); self.seq += 1
    def spread(self, fns, t0, t1):
        n = len(fns)
        for i, fn in enumerate(fns):
            self.at(t0 + (t1 - t0) * i / n, fn)
    def run_pass(self, dur, out, epi=None, R=8):
        t0 = self.t; self.t += dur
        rows = out.shape[0]
        if epi is not None:
            for r0 in range(0, rows, R):
                self.at(t0 + dur * (r0 + R - 0.5) / rows, lambda g, r0=r0: epi(r0, R))
        while True:
            due = sorted([x for x in self.tasks if x[0] < self.t], key=lambda x: x[:2])
            if not due: break
            x = due[0]
            self.tasks.remove(x)
            i = min(max(int((x[0] - t0) / dur * rows) // 8, 0), rows // 8 - 1)
            x[2](out[8 * i:8 * i + 8, 0:128])

class Head:
    def __init__(self, h, refs, scr, sc, z, never, tag):
        self.h = h; self.sc = sc; self.tag = tag
        self.q_ref, self.k_ref, self.v_ref, self.g_ref, self.o_ref, self.dq_ref, self.dk_ref, self.dv_ref = refs
        self.sb0, self.sb1, self.eb, self.db, self.xp, self.w, self.z, self.vc, self.ve, self.kc, self.ke, self.gc, self.ge, self.qc, self.qe = scr
        self.never = never
        self.sb = [self.sb0, self.sb1]
        self.zs = z
        self.m = [None, None]; self.l = [None, None]; self.b = [None, None]; self.t = [[None, None], [None, None]]; self.r = [None, None]; self.delta = [None, None]
    def gated(self, x, g):
        R, Cn = x.shape
        y = x.reshape(R // 8, 8, Cn)
        parts = [jnp.where(self.never[None], g[None], y[:, :, c:c + 128]) for c in range(0, Cn, 128)]
        return jnp.concatenate(parts, axis=2).reshape(R, Cn)
    def ld_e(self, j, r0, R, cs=slice(None)): return self.eb[self.zs[1], j, r0:r0 + R, cs]
    def ld_dp(self, j, r0, R): return self.db[self.zs[1], j, r0:r0 + R, :]
    def put_dp(self, items):
        for j, n, r, v in items:
            cs = slice(n * 128, (n + 1) * 128)
            self.db[self.zs[0], j, r:r + v.shape[0], cs] = v
            x = jnp.sum((v * self.ld_e(j, r, v.shape[0], cs)).reshape(v.shape[0] // 8, 8, 128), axis=0)
            self.t[j][n] = x if self.t[j][n] is None else self.t[j][n] + x
    def E0(self, ref, hr, fn, c_ref, e_ref, R=16):
        h = self.h
        def mk(r0):
            def f(g):
                x = []
                for rr in (r0, hr + r0):
                    y = ref[h, rr:rr + R, :].astype(f32)
                    x += [y[:, 0:hd], y[:, hd:]]
                d = fn(self.gated(x[0], g), x[1], x[2], self.gated(x[3], g))
                c_ref[self.zs[0], 0, r0:r0 + R, :] = jnp.concatenate([d["a"], d["b"]], axis=1).astype(bf)
                c_ref[self.zs[0], 1, r0:r0 + R, :] = jnp.concatenate([d["c"], d["d"]], axis=1).astype(bf)
                e_ref[self.zs[0], r0:r0 + R, :] = d["e"].astype(bf)
            return f
        return [mk(r0) for r0 in range(0, hr, R)]
    def op(self, ref, hr, c_ref, e_ref, nm, r0, r1, zi):
        h = self.h + self.zs[zi]
        z = self.zs[zi]
        if nm == "11": return ref[h, r0:r1, 0:hd]
        if nm == "22": return ref[h, hr + r0:hr + r1, hd:]
        if nm == "e": return e_ref[z, r0:r1, :]
        p, s = divmod("abcd".index(nm), 2)
        return c_ref[z, p, r0:r1, s * hd:(s + 1) * hd]
    def Vop(self, nm, r0=0, r1=hk, zi=1): return self.op(self.v_ref, hk, self.vc, self.ve, nm, r0, r1, zi)
    def Kop(self, nm, r0=0, r1=hk, zi=1): return self.op(self.k_ref, hk, self.kc, self.ke, nm, r0, r1, zi)
    def Gop(self, nm, r0=0, r1=hq, zi=1): return self.op(self.g_ref, hq, self.gc, self.ge, nm, r0, r1, zi)
    def Qop(self, nm, r0=0, r1=hq, zi=1): return self.op(self.q_ref, hq, self.qc, self.qe, nm, r0, r1, zi)
    def S(self, j):
        h = self.h
        s = tdot(f"{self.tag}s{j}", self.k_ref[h + self.zs[2 + j]], self.q_ref[h, j * hq:(j + 1) * hq, :], NT)
        sp = s * C2
        self.m[j] = jnp.broadcast_to(jnp.max(sp, axis=0, keepdims=True), (8, hq))
        def epi(r0, R):
            self.sb[j][self.zs[0], r0:r0 + R, :] = sp[r0:r0 + R]
        self.sc.run_pass(1024, s, epi)
    def dP(self):
        def unit(i, n, r0, r1):
            return tdot(f"{self.tag}dp{i}", self.Vop(BR[i - 1], r0, r1, 1 + n), self.Gop(AR[i - 1], n * 128, (n + 1) * 128), NT)
        za = self.zs[0]
        for n in range(2):
            cs = slice(n * 128, (n + 1) * 128)
            m2, m3, m4, m5 = [unit(i, n, 0, hk) for i in (2, 3, 4, 5)]
            def epi(r0, R):
                rs = slice(r0, r0 + R)
                self.put_dp([(0, n, hk + r0, m3[rs] + m5[rs]), (1, n, r0, m2[rs] + m4[rs])])
                self.xp[za, 0, r0:r0 + R, cs] = m4[rs] - m5[rs]
                self.xp[za, 1, r0:r0 + R, cs] = m3[rs] - m2[rs]
            self.sc.run_pass(512, m5, epi)
        H = hk // 2
        u = {}
        order = [(1,0,0),(6,0,0),(7,0,0),(1,0,1),(6,0,1),(7,0,1),(1,1,0),(6,1,0),(7,1,0),(1,1,1),(6,1,1),(7,1,1)]
        done = set()
        for p in range(3):
            for key in order[4 * p:4 * p + 4]:
                i, n, hh = key
                u[key] = unit(i, n, hh * H, (hh + 1) * H)
            todo = [(w, n, hh) for n in range(2) for hh in range(2) for w in (7, 6)
                    if (w, n, hh) in u and (1, n, hh) in u and (w, n, hh) not in done]
            done.update(todo)
            def epi(r0, R, todo=todo):
                rs = slice(r0, r0 + R)
                items = []
                for (w, n, hh) in todo:
                    cs = slice(n * 128, (n + 1) * 128)
                    rr = hh * H + r0
                    jj = 0 if w == 7 else 1
                    x = self.xp[self.zs[1], jj, rr:rr + R, cs]
                    items.append((jj, n, jj * hk + rr, x + u[(1, n, hh)][rs] + u[(w, n, hh)][rs]))
                self.put_dp(items)
            self.sc.run_pass(256, u[order[4 * p + 3]], epi)
        for j in range(2):
            t = jnp.sum(jnp.concatenate(self.t[j], axis=1), axis=0, keepdims=True)
            self.delta[j] = jnp.broadcast_to(t, (8, hq)) * self.r[j]
    def mm_nn(self, name, x_ref, Yop, out_ref, scale):
        h = self.h
        P = lambda i, r0=0, r1=hk: tdot(f"{self.tag}{name}{i}", x_ref[self.zs[1], NAMES.index(AR[i - 1]), r0:r1, :], Yop(BR[i - 1], zi=(2 if r0 == 0 else 3)), NN)
        fin = (lambda x: (x * scale).astype(bf)) if scale != 1 else (lambda x: x.astype(bf))
        m2 = P(2); m4 = P(4)
        self.sc.run_pass(512, m4)
        m3 = P(3); m5 = P(5)
        self.sc.run_pass(512, m5)
        m1 = P(1); m6 = P(6)
        out_ref[h, hk:, :] = fin(jnp.concatenate([m2 + m4, (m3 - m2) + (m1 + m6)], axis=1))
        self.sc.run_pass(512, m6)
        H = hk // 2
        m7 = jnp.concatenate([P(7, 0, H), P(7, H, hk)], axis=0)
        out_ref[h, 0:hk, :] = fin(jnp.concatenate([(m4 - m5) + (m1 + m7), m3 + m5], axis=1))
        self.sc.run_pass(256, m7[H:])
    def mm_tn(self, name, XT, Yop, out_ref, scale):
        h = self.h
        fin = (lambda x: (x * scale).astype(bf)) if scale != 1 else (lambda x: x.astype(bf))
        m = {}
        for i in TN_ORDER:
            m[i] = tdot(f"{self.tag}{name}{i}", XT[BR[i - 1]], Yop(AR[i - 1], zi=3), NN)
            if i == 6: out_ref[h, hq:, :] = fin(jnp.concatenate([m[3] + m[5], (m[3] - m[2]) + (m[1] + m[6])], axis=1))
            if i == 7: out_ref[h, 0:hq, :] = fin(jnp.concatenate([(m[4] - m[5]) + (m[1] + m[7]), m[2] + m[4]], axis=1))
            self.sc.run_pass(256, m[i])
    def T(self, x_ref):
        return {nm: x_ref[self.zs[2], NAMES.index(nm)].T for nm in [BR[i - 1] for i in TN_ORDER]}
    @staticmethod
    def bc(x, b, op):
        R = x.shape[0]
        return op(x.reshape(R // 8, 8, hq), b[None]).reshape(R, hq)
    def E1(self, j, R=32):
        def mk(r0):
            def f(g):
                e = jnp.exp2(self.bc(self.sb[j][self.zs[1], r0:r0 + R, :], self.gated(self.m[j], g), jnp.subtract))
                self.eb[self.zs[0], j, r0:r0 + R, :] = e
                e = jnp.sum(e.reshape(R // 8, 8, hq), axis=0)
                self.l[j] = e if self.l[j] is None else self.l[j] + e
                if r0 + R == Sk:
                    l = jnp.sum(self.l[j], axis=0, keepdims=True)
                    self.r[j] = jnp.broadcast_to(1.0 / l, (8, hq))
            return f
        return [mk(r0) for r0 in range(0, Sk, R)]
    def E2(self, R=8):
        def mk(r0):
            def f(g):
                r = [self.gated(x, g) for x in self.r]
                p = [[self.bc(self.ld_e(j, i * hk + r0, R), r[j], jnp.multiply) for j in range(2)] for i in range(2)]
                d = sset(p[0][0], p[0][1], p[1][0], p[1][1])
                for k, nm in enumerate(NAMES): self.w[self.zs[0], k, r0:r0 + R, :] = d[nm].astype(bf)
            return f
        return [mk(r0) for r0 in range(0, hk, R)]
    def E4(self, R=8):
        def mk(r0):
            def f(g):
                r = [self.gated(x, g) for x in self.r]
                z = [[None, None], [None, None]]
                for i in range(2):
                    for j in range(2):
                        p = self.bc(self.ld_e(j, i * hk + r0, R), r[j], jnp.multiply)
                        z[i][j] = p * self.bc(self.ld_dp(j, i * hk + r0, R), self.delta[j], jnp.subtract)
                d = sset(z[0][0], z[0][1], z[1][0], z[1][1])
                for k, nm in enumerate(NAMES): self.z[self.zs[0], k, r0:r0 + R, :] = d[nm].astype(bf)
            return f
        return [mk(r0) for r0 in range(0, hk, R)]

NS = 15
def _kernel(*refs):
    io, scr = refs[:8], refs[8:]
    pid = pl.program_id(0)
    zs = [pid >> 12, pid >> 13, pid >> 14, pid >> 15]
    never = jnp.full((8, 128), pid >> 16, jnp.int32) != 0
    sc = Sched()
    A = Head(0, io, scr[:NS], sc, zs, never, "A"); B = Head(1, io, scr[NS:], sc, zs, never, "B")
    P = 1792
    tSB, tdPA = 2048, 4096
    tdPB = tdPA + P; tdVA = tdPB + P; tOA = tdVA + P; tdKA = tOA + P; tdQA = tdKA + P
    tdVB = tdQA + P; tOB = tdVB + P; tdKB = tOB + P; tdQB = tdKB + P
    mg = 250
    def e0vg(X): return X.E0(X.g_ref, hq, sset, X.gc, X.ge) + X.E0(X.v_ref, hk, tset, X.vc, X.ve)
    def e0kq(X): return X.E0(X.q_ref, hq, sset, X.qc, X.qe) + X.E0(X.k_ref, hk, tset, X.kc, X.ke)
    sc.spread(e0vg(A), 0, 1100)
    sc.spread(A.E1(0), 1024 + 130, 2048 + 100)
    sc.spread(A.E1(1), 2048 + 130, 3072 + 100)
    sc.spread(B.E1(0), 3072 + 130, 4096 + 100)
    sc.spread(B.E1(1), 4096 + 130, 5120 + 100)
    sc.spread(e0vg(B), 2048, tdPB - mg - 512)
    sc.spread(A.E2(), 5120 + 100, tdVA - mg)
    sc.spread(A.E4(), tdVA + 1200, tdKA - mg)
    sc.spread(e0kq(A), tdVA, tdKA - mg)
    sc.spread(B.E2(), tdKA + 1200, tdVB - mg)
    sc.spread(B.E4(), tdVB + 1200, tdKB - mg)
    sc.spread(e0kq(B), tdVB, tdKB - mg)

    A.S(0); A.S(1); B.S(0); B.S(1); A.dP(); B.dP()
    for X in (A, B):
        WT = X.T(X.w)
        X.mm_nn("dv", X.w, X.Gop, X.dv_ref, 1)
        X.mm_tn("o", WT, X.Vop, X.o_ref, 1)
        ZT = X.T(X.z)
        X.mm_nn("dk", X.z, X.Qop, X.dk_ref, SCALE)
        X.mm_tn("dq", ZT, X.Kop, X.dq_ref, SCALE)
    assert not sc.tasks, len(sc.tasks)

V = pltpu.VMEM
_scr = [V((1, Sk, hq), f32), V((1, Sk, hq), f32), V((1, 2, Sk, hq), f32), V((1, 2, Sk, hq), f32), V((1, 2, hk, hq), f32), V((1, 7, hk, hq), bf), V((1, 7, hk, hq), bf),
        V((1, 2, hk, D), bf), V((1, hk, hd), bf), V((1, 2, hk, D), bf), V((1, hk, hd), bf),
        V((1, 2, hq, D), bf), V((1, hq, hd), bf), V((1, 2, hq, D), bf), V((1, hq, hd), bf)]

@jax.jit
def pallas_standalone__mha_softmax__near_ridge_kernel(q, k, v, grad_out):
    B, H = q.shape[:2]
    BH = B * H
    q3 = q.reshape(BH, Sq, D); k3 = k.reshape(BH, Sk, D); v3 = v.reshape(BH, Sk, D); g3 = grad_out.reshape(BH, Sq, D)
    qs = pl.BlockSpec((HPS, Sq, D), lambda i: (i, 0, 0))
    ks = pl.BlockSpec((HPS, Sk, D), lambda i: (i, 0, 0))
    o, dq, dk, dv = pl.pallas_call(
        _kernel,
        grid=(BH // HPS,),
        in_specs=[qs, ks, ks, qs],
        out_specs=[qs, qs, ks, ks],
        out_shape=[jax.ShapeDtypeStruct((BH, Sq, D), q.dtype), jax.ShapeDtypeStruct((BH, Sq, D), q.dtype),
                   jax.ShapeDtypeStruct((BH, Sk, D), q.dtype), jax.ShapeDtypeStruct((BH, Sk, D), q.dtype)],
        scratch_shapes=_scr * 2,
        compiler_params=pltpu.CompilerParams(dimension_semantics=("arbitrary",), vmem_limit_bytes=100 * 1024 * 1024),
        name="mha_kernel",
    )(q3, k3, v3, g3)
    return (o.reshape(B, H, Sq, D), dq.reshape(B, H, Sq, D), dk.reshape(B, H, Sk, D), dv.reshape(B, H, Sk, D))
```

```python
import jax
import jax.numpy as jnp
from jax import lax
import jax.experimental.pallas as pl
import jax.experimental.pallas.tpu as pltpu

NT = (((1,), (1,)), ((), ()))
NN = (((1,), (0,)), ((), ()))
f32 = jnp.float32
bf16 = jnp.bfloat16

SQ, SK, D = 512, 1024, 256
HQ, HK, HD = SQ // 2, SK // 2, D // 2
HEADS_PER_STEP = 2
SCALE = D ** -0.5
EXP2_SCALE = SCALE * 1.4426950408889634

NAMES = ["a", "b", "c", "d", "e", "11", "22"]
LHS_ROLE = ["a", "b", "11", "22", "c", "d", "e"]
RHS_ROLE = ["a", "11", "e", "d", "22", "c", "b"]
TN_ORDER = (2, 4, 3, 5, 1, 6, 7)

WIN = dict(e1=(180, 150), R1=8, vgA=(0, 1120), vgB=(2220, 5120), e2A=(5360, 7410), e4=(1090, 3130),
           q=(910, 1670), k=(4490, 5110), e2B=(1750, 3220))


def _dot(a, b, dims):
    return lax.dot_general(a, b, dims, preferred_element_type=f32)


def _combos(x11, x12, x21, x22):
    return [x11 + x22, x21 + x22, x11 + x12, x21 - x11, x12 - x22, x11, x22]


def _combos_t(x11, x12, x21, x22):
    return [x11 + x22, x12 + x22, x11 + x21, x12 - x11, x21 - x22, x11, x22]


def _cat(xs, axis):
    return lax.concatenate(xs, axis)


def _colsum8(x):
    return jnp.sum(x.reshape(x.shape[0] // 8, 8, x.shape[1]), axis=0)


def _out(left, right):
    return _cat([left, right], 1).astype(bf16)


class _Timeline:
    def __init__(self):
        self.t = 0
        self.tasks = []

    def spread(self, fns, t0, t1):
        for i, fn in enumerate(fns):
            self.tasks.append((t0 + (t1 - t0) * i / len(fns), len(self.tasks), fn))

    def mxu_pass(self, cycles, result):
        t0 = self.t
        self.t += cycles
        tiles = result.shape[0] // 8
        for t, _, fn in sorted((x for x in self.tasks if t0 <= x[0] < self.t), key=lambda x: x[:2]):
            i = min(int((t - t0) / cycles * tiles), tiles - 1)
            fn(lax.slice(result, (8 * i, 0), (8 * i + 8, 128)))


class _Head:
    def __init__(self, h, io, scratch, timeline, zeros, never):
        self.h, self.tl, self.z, self.never = h, timeline, zeros, never
        (self.q_ref, self.k_ref, self.v_ref, self.g_ref,
         self.dv_ref, self.o_ref, self.dk_ref, self.dq_ref) = io
        (s0, s1, self.e_buf, self.dp_buf, self.part_buf, self.p_ops, self.ds_ops,
         self.v4, self.v1, self.k4, self.k1, self.g4, self.g1, self.q4, self.q1) = scratch
        self.s_buf = [s0, s1]
        self.m = [None, None]
        self.l = [None, None]
        self.r = [None, None]
        self.rs = [None, None]
        self.t = [[None, None], [None, None]]
        self.delta = [None, None]

    def after(self, x, tile):
        return lax.select(self.never[x.shape], tile, x)

    def _operand(self, ref, half, four, one, name, r0, r1, zi):
        z = self.z[zi]
        if name == "11":
            return ref[self.h + z, r0:r1, 0:HD]
        if name == "22":
            return ref[self.h + z, half + r0:half + r1, HD:]
        if name == "e":
            return one[z, r0:r1, :]
        c = "abcd".index(name)
        return four[z, r0:r1, c * HD:(c + 1) * HD]

    def v_op(self, name, r0=0, r1=HK, zi=1):
        return self._operand(self.v_ref, HK, self.v4, self.v1, name, r0, r1, zi)

    def k_op(self, name, r0=0, r1=HK, zi=1):
        return self._operand(self.k_ref, HK, self.k4, self.k1, name, r0, r1, zi)

    def g_op(self, name, r0=0, r1=HQ, zi=1):
        return self._operand(self.g_ref, HQ, self.g4, self.g1, name, r0, r1, zi)

    def q_op(self, name, r0=0, r1=HQ, zi=1):
        return self._operand(self.q_ref, HQ, self.q4, self.q1, name, r0, r1, zi)

    def big_op(self, ops, name, r0, r1, zi):
        c = NAMES.index(name)
        return ops[self.z[zi], r0:r1, c * HQ:(c + 1) * HQ]

    def transposed(self, ops):
        return {n: self.big_op(ops, n, 0, HK, 2).T for n in [RHS_ROLE[i - 1] for i in TN_ORDER]}

    def scores(self, j):
        s = _dot(self.k_ref[self.h + self.z[2 + j]], self.q_ref[self.h, j * HQ:(j + 1) * HQ, :], NT)
        sp = s * EXP2_SCALE
        self.s_buf[j][self.z[0]] = sp
        self.m[j] = jnp.broadcast_to(jnp.max(sp, axis=0, keepdims=True), (8, HQ))
        self.tl.mxu_pass(1024, s)

    def _put_dp(self, j, n, row, val):
        cols = slice(n * 128, (n + 1) * 128)
        rows = slice(row, row + val.shape[0])
        self.dp_buf[self.z[0], j, rows, cols] = val
        x = _colsum8(val * self.e_buf[self.z[1], j, rows, cols])
        self.t[j][n] = x if self.t[j][n] is None else self.t[j][n] + x

    def dprobs(self):
        def unit(i, n, r0, r1):
            return _dot(self.v_op(RHS_ROLE[i - 1], r0, r1, 1 + n),
                        self.g_op(LHS_ROLE[i - 1], n * 128, (n + 1) * 128), NT)

        for n in range(2):
            cols = slice(n * 128, (n + 1) * 128)
            m2, m3, m4, m5 = [unit(i, n, 0, HK) for i in (2, 3, 4, 5)]
            self._put_dp(0, n, HK, m3 + m5)
            self._put_dp(1, n, 0, m2 + m4)
            self.part_buf[self.z[0], 0, :, cols] = m4 - m5
            self.part_buf[self.z[0], 1, :, cols] = m3 - m2
            self.tl.mxu_pass(512, m5)
        half = HK // 2
        order = [(i, n, s) for n in range(2) for s in range(2) for i in (1, 6, 7)]
        m, done = {}, set()
        for p in range(3):
            for i, n, s in order[4 * p:4 * p + 4]:
                m[i, n, s] = unit(i, n, s * half, (s + 1) * half)
            for n in range(2):
                for s in range(2):
                    for j, i in ((0, 7), (1, 6)):
                        if (i, n, s) in m and (1, n, s) in m and (i, n, s) not in done:
                            done.add((i, n, s))
                            x = self.part_buf[self.z[1], j, s * half:(s + 1) * half, n * 128:(n + 1) * 128]
                            self._put_dp(j, n, j * HK + s * half, x + m[1, n, s] + m[i, n, s])
            self.tl.mxu_pass(256, m[order[4 * p + 3]])
        for j in range(2):
            t = jnp.sum(_cat(self.t[j], 1), axis=0, keepdims=True)
            self.delta[j] = jnp.broadcast_to(t, (8, HQ)) * self.r[j]
            self.rs[j] = self.r[j] * SCALE

    def matmul_keys(self, ops, rhs_op, out_ref):
        def prod(i, r0=0, r1=HK):
            return _dot(self.big_op(ops, LHS_ROLE[i - 1], r0, r1, 1),
                        rhs_op(RHS_ROLE[i - 1], zi=(2 if r0 == 0 else 3)), NN)

        m2, m4 = prod(2), prod(4)
        self.tl.mxu_pass(512, m4)
        m3, m5 = prod(3), prod(5)
        self.tl.mxu_pass(512, m5)
        m1, m6 = prod(1), prod(6)
        out_ref[self.h, HK:, :] = _out(m2 + m4, (m3 - m2) + (m1 + m6))
        self.tl.mxu_pass(512, m6)
        m7 = [prod(7, 0, HK // 2), prod(7, HK // 2, HK)]
        out_ref[self.h, 0:HK, :] = _out((m4 - m5) + (m1 + _cat(m7, 0)), m3 + m5)
        self.tl.mxu_pass(256, m7[1])

    def matmul_queries(self, ops_t, rhs_op, out_ref):
        m = {}
        for i in TN_ORDER:
            m[i] = _dot(ops_t[RHS_ROLE[i - 1]], rhs_op(LHS_ROLE[i - 1], zi=3), NN)
            if i == 6:
                out_ref[self.h, HQ:, :] = _out(m[3] + m[5], (m[3] - m[2]) + (m[1] + m[6]))
            if i == 7:
                out_ref[self.h, 0:HQ, :] = _out((m[4] - m[5]) + (m[1] + m[7]), m[2] + m[4])
            self.tl.mxu_pass(256, m[i])

    def input_combos(self, ref, half, fn, four, one, rows=16):
        def strip(r0):
            def run(tile):
                tile = _cat([tile] * (rows // 8), 0)
                top = ref[self.h, r0:r0 + rows, :].astype(f32)
                bot = ref[self.h, half + r0:half + r0 + rows, :].astype(f32)
                c = fn(self.after(top[:, 0:HD], tile), top[:, HD:], bot[:, 0:HD], self.after(bot[:, HD:], tile))
                four[self.z[0], r0:r0 + rows, :] = _cat(c[0:4], 1).astype(bf16)
                one[self.z[0], r0:r0 + rows, :] = c[4].astype(bf16)
            return run
        return [strip(r0) for r0 in range(0, half, rows)]

    def exponentials(self, j, rows):
        def strip(r0):
            def run(tile):
                m = self.after(self.m[j], _cat([tile, tile], 1))
                e = jnp.exp2(self.s_buf[j][self.z[1], r0:r0 + rows, :] - _cat([m] * (rows // 8), 0))
                self.e_buf[self.z[0], j, r0:r0 + rows, :] = e
                e = _colsum8(e)
                self.l[j] = e if self.l[j] is None else self.l[j] + e
                if r0 + rows == SK:
                    l = jnp.sum(self.l[j], axis=0, keepdims=True)
                    self.r[j] = jnp.broadcast_to(1.0 / l, (8, HQ))
            return run
        return [strip(r0) for r0 in range(0, SK, rows)]

    def prob_combos(self, grad):
        def strip(r0):
            def run(tile):
                tile = _cat([tile, tile], 1)
                r = [self.after(x, tile) for x in (self.rs if grad else self.r)]
                x = []
                for i in range(2):
                    for j in range(2):
                        rows = slice(i * HK + r0, i * HK + r0 + 8)
                        p = self.e_buf[self.z[1], j, rows, :] * r[j]
                        x.append(p * (self.dp_buf[self.z[1], j, rows, :] - self.delta[j]) if grad else p)
                ops = self.ds_ops if grad else self.p_ops
                ops[self.z[0], r0:r0 + 8, :] = _cat(_combos(*x), 1).astype(bf16)
            return run
        return [strip(r0) for r0 in range(0, HK, 8)]


def _kernel(*refs):
    io, scratch = refs[:8], refs[8:]
    step = pl.program_id(0)
    zeros = [step >> 12, step >> 13, step >> 14, step >> 15]
    never = {s: jnp.full(s, step >> 16, jnp.int32) != 0 for s in ((8, 256), (16, 128))}
    tl = _Timeline()
    n = len(scratch) // 2
    a = _Head(0, io, scratch[:n], tl, zeros, never)
    b = _Head(1, io, scratch[n:], tl, zeros, never)

    phase = 1792
    t_a = 4096 + 2 * phase
    t_b = t_a + 4 * phase
    e0, e1 = WIN["e1"]
    for x, key in ((a, "vgA"), (b, "vgB")):
        tl.spread(x.input_combos(x.g_ref, HQ, _combos, x.g4, x.g1)
                  + x.input_combos(x.v_ref, HK, _combos_t, x.v4, x.v1), *WIN[key])
    for i, (x, j) in enumerate(((a, 0), (a, 1), (b, 0), (b, 1))):
        tl.spread(x.exponentials(j, WIN["R1"]), 1024 * (i + 1) + e0, 1024 * (i + 2) + e1)
    tl.spread(a.prob_combos(False), *WIN["e2A"])
    tl.spread(b.prob_combos(False), *[t_a + 2 * phase + t for t in WIN["e2B"]])
    for x, t0 in ((a, t_a), (b, t_b)):
        tl.spread(x.prob_combos(True), *[t0 + t for t in WIN["e4"]])
        tl.spread(x.input_combos(x.q_ref, HQ, _combos, x.q4, x.q1), *[t0 + t for t in WIN["q"]])
        tl.spread(x.input_combos(x.k_ref, HK, _combos_t, x.k4, x.k1), *[t0 + t for t in WIN["k"]])

    for x in (a, b):
        x.scores(0)
        x.scores(1)
    a.dprobs()
    b.dprobs()
    for x in (a, b):
        p_t = x.transposed(x.p_ops)
        x.matmul_keys(x.p_ops, x.g_op, x.dv_ref)
        x.matmul_queries(p_t, x.v_op, x.o_ref)
        ds_t = x.transposed(x.ds_ops)
        x.matmul_keys(x.ds_ops, x.q_op, x.dk_ref)
        x.matmul_queries(ds_t, x.k_op, x.dq_ref)


def _scratch_per_head():
    v = pltpu.VMEM
    return [
        v((1, SK, HQ), f32), v((1, SK, HQ), f32),
        v((1, 2, SK, HQ), f32), v((1, 2, SK, HQ), f32),
        v((1, 2, HK, HQ), f32),
        v((1, HK, 7 * HQ), bf16), v((1, HK, 7 * HQ), bf16),
        v((1, HK, 4 * HD), bf16), v((1, HK, HD), bf16),
        v((1, HK, 4 * HD), bf16), v((1, HK, HD), bf16),
        v((1, HQ, 4 * HD), bf16), v((1, HQ, HD), bf16),
        v((1, HQ, 4 * HD), bf16), v((1, HQ, HD), bf16),
    ]


@jax.jit
def pallas_standalone__mha_softmax__near_ridge_kernel(
    q: jax.Array,
    k: jax.Array,
    v: jax.Array,
    grad_out: jax.Array,
):
    batch, heads = q.shape[:2]
    bh = batch * heads
    q_spec = pl.BlockSpec((HEADS_PER_STEP, SQ, D), lambda i: (i, 0, 0))
    k_spec = pl.BlockSpec((HEADS_PER_STEP, SK, D), lambda i: (i, 0, 0))
    q_like = jax.ShapeDtypeStruct((bh, SQ, D), q.dtype)
    k_like = jax.ShapeDtypeStruct((bh, SK, D), q.dtype)
    dv, o, dk, dq = pl.pallas_call(
        _kernel,
        grid=(bh // HEADS_PER_STEP,),
        in_specs=[q_spec, k_spec, k_spec, q_spec],
        out_specs=[k_spec, q_spec, k_spec, q_spec],
        out_shape=[k_like, q_like, k_like, q_like],
        scratch_shapes=_scratch_per_head() * HEADS_PER_STEP,
        compiler_params=pltpu.CompilerParams(
            dimension_semantics=("arbitrary",),
            vmem_limit_bytes=100 * 1024 * 1024,
            disable_bounds_checks=True,
        ),
        name="mha_kernel",
    )(q.reshape(bh, SQ, D), k.reshape(bh, SK, D), v.reshape(bh, SK, D), grad_out.reshape(bh, SQ, D))
    return (o.reshape(q.shape), dq.reshape(q.shape), dk.reshape(k.shape), dv.reshape(k.shape))
```

```python
import jax
import jax.numpy as jnp
from jax import lax
import jax.experimental.pallas as pl
import jax.experimental.pallas.tpu as pltpu

NT = (((1,), (1,)), ((), ()))
NN = (((1,), (0,)), ((), ()))
f32 = jnp.float32
bf16 = jnp.bfloat16

SQ, SK, D = 512, 1024, 256
HQ, HK, HD = SQ // 2, SK // 2, D // 2
HEADS_PER_STEP = 2
SCALE = D ** -0.5
EXP2_SCALE = SCALE * 1.4426950408889634

NAMES = ["a", "b", "c", "d", "e", "11", "22"]
LHS_ROLE = ["a", "b", "11", "22", "c", "d", "e"]
RHS_ROLE = ["a", "11", "e", "d", "22", "c", "b"]
TN_ORDER = (2, 4, 3, 5, 1, 6, 7)

LAM = [-1.0, -0.28125, 0.28125, 1.0]
PAIRS = [(0, 1), (2, 3), (0, 2), (1, 3), (0, 3), (1, 2)]
RIDERS = [("u", 1), ("u", 2), ("w", 2), ("u", 3), ("w", 3), ("w", 1)]
HK_OPS = [("u", 0), ("w", 0)] + [o for p, e in zip(PAIRS, RIDERS) for o in (("x",) + p, ("y",) + p, ("z",) + p, e)]
K_OPS = [o for o in HK_OPS if o[0] != "u"]
Q_OPS = [o for o in HK_OPS if o[0] != "w"]
KB, QB = SK // 4, SQ // 4

PHASES = ["SA", "SB", "dPA", "dPB", "dVA", "OA", "dVB", "OB", "dKA", "dQA", "dKB", "dQB"]
BIN = 128
BASE = {
    "S": ([100] * 16, [32] * 16),
    "dP": ([150] * 8 + [135, 150, 200, 200, 200, 200], [64] * 8 + [50] * 6),
    "dV": ([100, 120, 120, 150, 110, 120, 105, 150, 145, 155, 155, 150, 200, 175],
           [72, 76, 76, 80, 85, 60, 45, 45, 32, 32, 32, 32, 30, 30]),
    "O": ([110, 70, 65, 70, 65, 75, 75, 80, 60, 60, 110, 130, 110, 150], [20] + [16] * 7 + [25] * 6),
    "dK": ([140, 260, 290, 140, 170, 310, 310, 200, 220, 330, 350, 310, 320],
           [100, 90, 97, 85, 75, 80, 80, 42, 26, 35, 32, 32, 32]),
    "dQ": ([110, 70, 300, 70, 125, 100, 390, 80, 220, 100, 420, 150, 400],
           [14, 13, 70, 18, 37, 24, 84, 18, 59, 22, 30, 30, 45]),
}
LEAD_IN = [60, 100, 130, 130]
PLAN = dict(wv=1.0, pw=4, margin=300, lag=256, p_from=3400, ds_in=("O", "dQ"), qk_in=("S", "dP", "dV", "dK"))


def _dot(a, b, dims):
    return lax.dot_general(a, b, dims, preferred_element_type=f32)


def _combos(x11, x12, x21, x22):
    return [x11 + x22, x21 + x22, x11 + x12, x21 - x11, x12 - x22, x11, x22]


def _combos_t(x11, x12, x21, x22):
    return [x11 + x22, x12 + x22, x11 + x21, x12 - x11, x21 - x22, x11, x22]


def _cat(xs, axis):
    return lax.concatenate(xs, axis)


def _colsum8(x):
    return jnp.sum(x.reshape(x.shape[0] // 8, 8, x.shape[1]), axis=0)


def _out(left, right):
    return _cat([left, right], 1).astype(bf16)


def _acc(acc, key, x):
    acc[key] = x if key not in acc else acc[key] + x


class _Scaled:
    def __init__(self, x):
        self.m = {1.0: x}

    def axpy(self, y, c):
        a = abs(c)
        if a not in self.m:
            self.m[a] = self.m[1.0] * a
        if y is None:
            return self.m[a] if c > 0 else -self.m[a]
        return y + self.m[a] if c > 0 else y - self.m[a]


class _Timeline:
    def __init__(self):
        self.t = 0
        self.start, self.kind, self.valu, self.vst = {}, [], [], []
        for name in PHASES:
            self.start[name] = BIN * len(self.valu)
            valu, vst = BASE[name[:-1]]
            if name[:-1] in ("dV", "dK"):
                for n, x in enumerate(LEAD_IN):
                    self.valu[n - len(LEAD_IN)] += x
                    self.vst[n - len(LEAD_IN)] += x / 6
            self.kind += [name[:-1]] * len(valu)
            self.valu += valu
            self.vst += vst
        self.bins = [[] for _ in self.valu]
        self.groups, self.movable, self.tasks = [], {}, []

    def _put(self, k, group, valu, vst):
        self.valu[k] += valu
        self.vst[k] += vst
        self.bins[k].append((group, valu))

    def spread(self, fns, t0, t1, valu, vst):
        self.groups.append(fns)
        for i in range(len(fns)):
            self._put(int(t0 + (t1 - t0) * i / len(fns)) // BIN, len(self.groups) - 1, valu, vst)

    def fill(self, fns, t0, t1, valu, vst, kinds=None):
        self.groups.append(fns)
        ks = [k for k in range(-(-t0 // BIN), t1 // BIN) if kinds is None or self.kind[k] in kinds]
        self.movable[len(self.groups) - 1] = (ks, vst)
        for _ in fns:
            k = min(ks, key=lambda k: max((self.valu[k] + valu) / 4, PLAN["wv"] * (self.vst[k] + vst)))
            self._put(k, len(self.groups) - 1, valu, vst)

    def _rebalance(self):
        cost = lambda valu, vst: (valu / 400) ** PLAN["pw"] + (PLAN["wv"] * vst / 100) ** PLAN["pw"]
        while True:
            best = None
            for k, items in enumerate(self.bins):
                for g, valu in sorted(set(items)):
                    if g not in self.movable:
                        continue
                    ks, vst = self.movable[g]
                    gain = cost(self.valu[k], self.vst[k]) - cost(self.valu[k] - valu, self.vst[k] - vst)
                    for k2 in ks:
                        d = gain - (cost(self.valu[k2] + valu, self.vst[k2] + vst) - cost(self.valu[k2], self.vst[k2]))
                        if k2 != k and d > 1e-9 and (best is None or d > best[0]):
                            best = (d, k, k2, g, valu, vst)
            if best is None:
                return
            _, k, k2, g, valu, vst = best
            self.bins[k].remove((g, valu))
            self.valu[k] -= valu
            self.vst[k] -= vst
            self._put(k2, g, valu, vst)

    def finish(self):
        self._rebalance()
        times = [[] for _ in self.groups]
        for k, items in enumerate(self.bins):
            by = {}
            for g, valu in items:
                by.setdefault(g, []).append(valu)
            seq = sorted(((n + 0.5) / len(v), g, v[n]) for g, v in by.items() for n in range(len(v)))
            total, cum, last = sum(x[2] + 8 for x in seq), 0, -8
            for _, g, valu in seq:
                last = max(int(cum / total * BIN) // 8 * 8, last + 8)
                assert last < BIN
                times[g].append(k * BIN + last)
                cum += valu + 8
        for g, fns in enumerate(self.groups):
            self.tasks += list(zip(sorted(times[g]), fns))
        self.tasks.sort(key=lambda x: x[0])

    def mxu_pass(self, cycles, result):
        t0 = self.t
        self.t += cycles
        for t, fn in self.tasks:
            if t0 <= t < self.t:
                i = (t - t0) * result.shape[0] // cycles // 8
                fn(lax.slice(result, (8 * i, 0), (8 * i + 8, 128)))


class _Head:
    def __init__(self, h, io, scratch, timeline, zeros, never):
        self.h, self.tl, self.z, self.never = h, timeline, zeros, never
        (self.q_ref, self.k_ref, self.v_ref, self.g_ref,
         self.dv_ref, self.o_ref, self.dk_ref, self.dq_ref) = io
        (s0, s1, self.e_buf, self.dp_buf, self.part_buf, self.p_ops, self.ds_ops,
         self.v4, self.v1, self.k_ops, self.g4, self.g1, self.q_ops) = scratch
        self.s_buf = [s0, s1]
        self.m = [None, None]
        self.l = [None, None]
        self.r = [None, None]
        self.rs = [None, None]
        self.t = [[None, None], [None, None]]
        self.delta = [None, None]

    def after(self, x, tile):
        return lax.select(self.never[x.shape], tile, x)

    def _operand(self, ref, half, four, one, name, r0, r1, zi):
        z = self.z[zi]
        if name == "11":
            return ref[self.h + z, r0:r1, 0:HD]
        if name == "22":
            return ref[self.h + z, half + r0:half + r1, HD:]
        if name == "e":
            return one[z, r0:r1, :]
        c = "abcd".index(name)
        return four[z, r0:r1, c * HD:(c + 1) * HD]

    def v_op(self, name, r0=0, r1=HK, zi=1):
        return self._operand(self.v_ref, HK, self.v4, self.v1, name, r0, r1, zi)

    def g_op(self, name, r0=0, r1=HQ, zi=1):
        return self._operand(self.g_ref, HQ, self.g4, self.g1, name, r0, r1, zi)

    def p_op(self, name, r0, r1, zi):
        c = NAMES.index(name)
        return self.p_ops[self.z[zi], r0:r1, c * HQ:(c + 1) * HQ]

    def k_op(self, o):
        z = self.z[3]
        if o[0] == "u":
            return self.k_ref[self.h + z, o[1] * KB:(o[1] + 1) * KB, 0:HD]
        c = K_OPS.index(o)
        return self.k_ops[z, :, c * HD:(c + 1) * HD]

    def q_op(self, o, zi):
        z = self.z[zi]
        if o[0] == "w":
            return self.q_ref[self.h + z, o[1] * QB:(o[1] + 1) * QB, HD:]
        c = Q_OPS.index(o)
        return self.q_ops[z, :, c * HD:(c + 1) * HD]

    def ds_op(self, o, r0, r1):
        c = HK_OPS.index(o)
        return self.ds_ops[self.z[1], r0:r1, c * 128:(c + 1) * 128]

    def scores(self, j):
        s = _dot(self.k_ref[self.h + self.z[2 + j]], self.q_ref[self.h, j * HQ:(j + 1) * HQ, :], NT)
        sp = s * EXP2_SCALE
        self.s_buf[j][self.z[0]] = sp
        self.m[j] = jnp.broadcast_to(jnp.max(sp, axis=0, keepdims=True), (8, HQ))
        self.tl.mxu_pass(1024, s)

    def _put_dp(self, j, n, row, val):
        cols = slice(n * 128, (n + 1) * 128)
        rows = slice(row, row + val.shape[0])
        self.dp_buf[self.z[0], j, rows, cols] = val
        x = _colsum8(val * self.e_buf[self.z[1], j, rows, cols])
        self.t[j][n] = x if self.t[j][n] is None else self.t[j][n] + x

    def dprobs(self):
        def unit(i, n, r0, r1):
            return _dot(self.v_op(RHS_ROLE[i - 1], r0, r1, 1 + n),
                        self.g_op(LHS_ROLE[i - 1], n * 128, (n + 1) * 128), NT)

        for n in range(2):
            cols = slice(n * 128, (n + 1) * 128)
            m2, m3, m4, m5 = [unit(i, n, 0, HK) for i in (2, 3, 4, 5)]
            self._put_dp(0, n, HK, m3 + m5)
            self._put_dp(1, n, 0, m2 + m4)
            self.part_buf[self.z[0], 0, :, cols] = m4 - m5
            self.part_buf[self.z[0], 1, :, cols] = m3 - m2
            self.tl.mxu_pass(512, m5)
        half = HK // 2
        order = [(i, n, s) for n in range(2) for s in range(2) for i in (1, 6, 7)]
        m, done = {}, set()
        for p in range(3):
            for i, n, s in order[4 * p:4 * p + 4]:
                m[i, n, s] = unit(i, n, s * half, (s + 1) * half)
            for n in range(2):
                for s in range(2):
                    for j, i in ((0, 7), (1, 6)):
                        if (i, n, s) in m and (1, n, s) in m and (i, n, s) not in done:
                            done.add((i, n, s))
                            x = self.part_buf[self.z[1], j, s * half:(s + 1) * half, n * 128:(n + 1) * 128]
                            self._put_dp(j, n, j * HK + s * half, x + m[1, n, s] + m[i, n, s])
            self.tl.mxu_pass(256, m[order[4 * p + 3]])
        for j in range(2):
            t = jnp.sum(_cat(self.t[j], 1), axis=0, keepdims=True)
            self.delta[j] = jnp.broadcast_to(t, (8, HQ)) * self.r[j]
            self.rs[j] = self.r[j] * SCALE

    def dvalues(self):
        self.p_t = {n: self.p_op(n, 0, HK, 2).T for n in [RHS_ROLE[i - 1] for i in TN_ORDER]}

        def prod(i, r0=0, r1=HK):
            return _dot(self.p_op(LHS_ROLE[i - 1], r0, r1, 1),
                        self.g_op(RHS_ROLE[i - 1], zi=(2 if r0 == 0 else 3)), NN)

        m2, m4 = prod(2), prod(4)
        self.tl.mxu_pass(512, m4)
        m3, m5 = prod(3), prod(5)
        self.tl.mxu_pass(512, m5)
        m1, m6 = prod(1), prod(6)
        self.dv_ref[self.h, HK:, :] = _out(m2 + m4, (m3 - m2) + (m1 + m6))
        self.tl.mxu_pass(512, m6)
        m7 = [prod(7, 0, HK // 2), prod(7, HK // 2, HK)]
        self.dv_ref[self.h, 0:HK, :] = _out((m4 - m5) + (m1 + _cat(m7, 0)), m3 + m5)
        self.tl.mxu_pass(256, m7[1])

    def output(self):
        m = {}
        for i in TN_ORDER:
            m[i] = _dot(self.p_t[RHS_ROLE[i - 1]], self.v_op(LHS_ROLE[i - 1], zi=3), NN)
            if i == 6:
                self.o_ref[self.h, HQ:, :] = _out(m[3] + m[5], (m[3] - m[2]) + (m[1] + m[6]))
            if i == 7:
                self.o_ref[self.h, 0:HQ, :] = _out((m[4] - m[5]) + (m[1] + m[7]), m[2] + m[4])
            self.tl.mxu_pass(256, m[i])

    def dkeys(self):
        self.ds_t = [self.ds_ops[self.z[2], :, m * 256:(m + 1) * 256].T for m in range(13)]
        acc = {}

        def prod(o, r0=0, r1=KB, zi=2):
            return _dot(self.ds_op(o, r0, r1), self.q_op(o, zi), NN)

        def single(o, r):
            if o[0] == "u":
                _acc(acc, (o[1], 0), r)
            else:
                acc[o[1], 0] = _Scaled(r).axpy(acc.get((o[1], 0)), -LAM[o[1]])
                _acc(acc, (o[1], 1), r)

        first = [[prod(o, 0, KB // 2), prod(o, KB // 2, KB, 3)] for o in HK_OPS[0:2]]
        for o, r in zip(HK_OPS[0:2], first):
            single(o, _cat(r, 0))
        self.tl.mxu_pass(128, first[1][1])
        left = [3] * 4
        for p, ((i, j), rider) in enumerate(zip(PAIRS, RIDERS)):
            x, y, z, e = [prod(o) for o in HK_OPS[2 + 4 * p:6 + 4 * p]]
            c = x + (y + z)
            sign = 1.0 if LAM[j] > 0 else -1.0
            if LAM[i] == -LAM[j]:
                u = _Scaled(y - z).axpy(None, LAM[j])
            else:
                u = _Scaled(z).axpy(_Scaled(y).axpy(None, sign * LAM[j]), sign * LAM[i])
            single(rider, e)
            sx = _Scaled(x)
            for t in (i, j):
                _acc(acc, (t, 1), c)
                acc[t, 0] = _Scaled(sx.axpy(u, sign * LAM[t])).axpy(acc.get((t, 0)), -sign)
                left[t] -= 1
                if left[t] == 0:
                    self.dk_ref[self.h, t * KB:(t + 1) * KB, :] = _out(acc[t, 0], acc[t, 1])
            self.tl.mxu_pass(256, e)

    def dqueries(self):
        acc = {}

        def prods(m):
            return [_dot(self.ds_t[m][s * QB:(s + 1) * QB], self.k_op(HK_OPS[2 * m + s]), NN) for s in range(2)]

        def single(o, r):
            if o[0] == "u":
                _acc(acc, (o[1], 0), r)
                acc[o[1], 1] = _Scaled(r).axpy(acc.get((o[1], 1)), LAM[o[1]])
            else:
                _acc(acc, (o[1], 1), r)

        first = prods(0)
        for o, r in zip(HK_OPS[0:2], first):
            single(o, r)
        self.tl.mxu_pass(128, first[1])
        left = [3] * 4
        for p, ((i, j), rider) in enumerate(zip(PAIRS, RIDERS)):
            a = 1.0 / (LAM[i] - LAM[j])
            x, y = prods(1 + 2 * p)
            self.tl.mxu_pass(128, y)
            z, e = prods(2 + 2 * p)
            c = (x - (y + z)) * a
            if LAM[i] == -LAM[j]:
                w = (y - z) * (a * LAM[i])
            else:
                w = y * (a * LAM[i]) + z * (a * LAM[j])
            sx = _Scaled(x)
            single(rider, e)
            _acc(acc, (i, 0), c)
            acc[j, 0] = _Scaled(c).axpy(acc.get((j, 0)), -1.0)
            acc[i, 1] = _Scaled(sx.axpy(w, -a * LAM[i])).axpy(acc.get((i, 1)), -1.0)
            _acc(acc, (j, 1), sx.axpy(w, -a * LAM[j]))
            for t in (i, j):
                left[t] -= 1
                if left[t] == 0:
                    self.dq_ref[self.h, t * QB:(t + 1) * QB, :] = _out(acc[t, 0], acc[t, 1])
            self.tl.mxu_pass(128, e)

    def input_combos(self, ref, half, fn, four, one, rows=16):
        def strip(r0):
            def run(tile):
                tile = _cat([tile] * (rows // 8), 0)
                top = ref[self.h, r0:r0 + rows, :].astype(f32)
                bot = ref[self.h, half + r0:half + r0 + rows, :].astype(f32)
                c = fn(self.after(top[:, 0:HD], tile), top[:, HD:], bot[:, 0:HD], self.after(bot[:, HD:], tile))
                four[self.z[0], r0:r0 + rows, :] = _cat(c[0:4], 1).astype(bf16)
                one[self.z[0], r0:r0 + rows, :] = c[4].astype(bf16)
            return run
        return [strip(r0) for r0 in range(0, half, rows)]

    def exponentials(self, j, rows):
        def strip(r0):
            def run(tile):
                m = self.after(self.m[j], _cat([tile, tile], 1))
                e = jnp.exp2(self.s_buf[j][self.z[1], r0:r0 + rows, :] - _cat([m] * (rows // 8), 0))
                self.e_buf[self.z[0], j, r0:r0 + rows, :] = e
                e = _colsum8(e)
                self.l[j] = e if self.l[j] is None else self.l[j] + e
                if r0 + rows == SK:
                    l = jnp.sum(self.l[j], axis=0, keepdims=True)
                    self.r[j] = jnp.broadcast_to(1.0 / l, (8, HQ))
            return run
        return [strip(r0) for r0 in range(0, SK, rows)]

    def prob_combos(self):
        def strip(r0):
            def run(tile):
                tile = _cat([tile, tile], 1)
                r = [self.after(x, tile) for x in self.r]
                p = [self.e_buf[self.z[1], j, i * HK + r0:i * HK + r0 + 8, :] * r[j] for i in range(2) for j in range(2)]
                self.p_ops[self.z[0], r0:r0 + 8, :] = _cat(_combos(*p), 1).astype(bf16)
            return run
        return [strip(r0) for r0 in range(0, HK, 8)]

    def dscore_combos(self):
        def strip(r0):
            def run(tile):
                tile = _cat([tile, tile], 1)
                r = [self.after(x, tile) for x in self.rs]
                ds = {}
                for kb in range(4):
                    rows = slice(kb * KB + r0, kb * KB + r0 + 8)
                    for j in range(2):
                        x = (self.e_buf[self.z[1], j, rows, :] * r[j]) * (self.dp_buf[self.z[1], j, rows, :] - self.delta[j])
                        ds[2 * j, kb], ds[2 * j + 1, kb] = x[:, 0:128], x[:, 128:]
                d = {}
                for i in range(4):
                    o = [t for t in range(4) if t != i]
                    d["u", i] = (ds[0, i] + ds[1, i]) + (ds[2, i] + ds[3, i])
                    d["w", i] = (ds[i, i] - ds[i, o[0]]) - (ds[i, o[1]] + ds[i, o[2]])
                for i, j in PAIRS:
                    d["x", i, j], d["y", i, j], d["z", i, j] = ds[i, j] + ds[j, i], ds[j, i], ds[i, j]
                self.ds_ops[self.z[0], r0:r0 + 8, :] = _cat([d[o] for o in HK_OPS], 1).astype(bf16)
            return run
        return [strip(r0) for r0 in range(0, KB, 8)]

    def key_combos(self):
        def strip(r0):
            def run(tile):
                x = [self.k_ref[self.h, i * KB + r0:i * KB + r0 + 8, :].astype(f32) for i in range(4)]
                k1 = [self.after(y[:, 0:HD], tile) for y in x]
                k2 = [y[:, HD:] for y in x]
                d = {("w", i): _Scaled(k1[i]).axpy(k2[i], -LAM[i]) for i in range(4)}
                for i, j in PAIRS:
                    s1, s2 = _Scaled(k1[i] + k1[j]), k2[i] + k2[j]
                    d["x", i, j] = d["w", i] + d["w", j]
                    d["y", i, j] = s1.axpy(s2, -LAM[j])
                    d["z", i, j] = s1.axpy(s2, -LAM[i])
                self.k_ops[self.z[0], r0:r0 + 8, :] = _cat([d[o] for o in K_OPS], 1).astype(bf16)
            return run
        return [strip(r0) for r0 in range(0, KB, 8)]

    def query_combos(self):
        def strip(r0):
            def run(tile):
                x = [self.q_ref[self.h, i * QB + r0:i * QB + r0 + 8, :].astype(f32) for i in range(4)]
                q1 = [y[:, 0:HD] for y in x]
                q2 = [self.after(y[:, HD:], tile) for y in x]
                d = {("u", i): _Scaled(q2[i]).axpy(q1[i], LAM[i]) for i in range(4)}
                for i, j in PAIRS:
                    a = 1.0 / (LAM[i] - LAM[j])
                    d1, d2 = (q1[j] - q1[i]) * a, _Scaled(q2[j] - q2[i])
                    d["x", i, j] = (d["u", i] - d["u", j]) * a
                    d["y", i, j] = d2.axpy(d1, a * LAM[i])
                    d["z", i, j] = d2.axpy(d1, a * LAM[j])
                self.q_ops[self.z[0], r0:r0 + 8, :] = _cat([d[o] for o in Q_OPS], 1).astype(bf16)
            return run
        return [strip(r0) for r0 in range(0, QB, 8)]


def _kernel(*refs):
    io, scratch = refs[:8], refs[8:]
    step = pl.program_id(0)
    zeros = [step >> 12, step >> 13, step >> 14, step >> 15]
    never = {s: jnp.full(s, step >> 16, jnp.int32) != 0 for s in ((8, 256), (16, 128), (8, 128))}
    tl = _Timeline()
    n = len(scratch) // 2
    heads = {"A": _Head(0, io, scratch[:n], tl, zeros, never), "B": _Head(1, io, scratch[n:], tl, zeros, never)}
    a, b = heads["A"], heads["B"]

    at, margin, lag = tl.start, PLAN["margin"], PLAN["lag"]
    for i, (x, j) in enumerate(((a, 0), (a, 1), (b, 0), (b, 1))):
        tl.spread(x.exponentials(j, 16), 1024 * (i + 1) + lag, 1024 * (i + 2) + lag, 10.8, 4)
    for h, x in heads.items():
        tl.fill(x.dscore_combos(), at["dP" + h] + 1942, at["dK" + h] - margin, 95, 13, PLAN["ds_in"])
    tl.fill(a.prob_combos(), PLAN["p_from"], at["dVA"] - margin, 29, 7)
    for h, x in heads.items():
        tl.fill(x.input_combos(x.g_ref, HQ, _combos, x.g4, x.g1) + x.input_combos(x.v_ref, HK, _combos_t, x.v4, x.v1),
                0, at["dP" + h] - margin, 28, 5.5)
    for h, x in heads.items():
        tl.fill(x.query_combos(), 0, at["dK" + h] - margin, 81, 11, PLAN["qk_in"])
    for h, x in heads.items():
        tl.fill(x.key_combos(), 0, at["dQ" + h] - margin, 62, 11, PLAN["qk_in"])
    tl.fill(b.prob_combos(), at["dVA"], at["dVB"] - margin, 29, 7)
    tl.finish()

    for name in PHASES:
        x = heads[name[-1]]
        if name[:-1] == "S":
            x.scores(0)
            x.scores(1)
        else:
            {"dP": x.dprobs, "dV": x.dvalues, "O": x.output, "dK": x.dkeys, "dQ": x.dqueries}[name[:-1]]()


def _scratch_per_head():
    v = pltpu.VMEM
    return [
        v((1, SK, HQ), f32), v((1, SK, HQ), f32),
        v((1, 2, SK, HQ), f32), v((1, 2, SK, HQ), f32),
        v((1, 2, HK, HQ), f32),
        v((1, HK, 7 * HQ), bf16), v((1, KB, 26 * 128), bf16),
        v((1, HK, 4 * HD), bf16), v((1, HK, HD), bf16),
        v((1, KB, 22 * HD), bf16),
        v((1, HQ, 4 * HD), bf16), v((1, HQ, HD), bf16),
        v((1, QB, 22 * HD), bf16),
    ]


@jax.jit
def pallas_standalone__mha_softmax__near_ridge_kernel(
    q: jax.Array,
    k: jax.Array,
    v: jax.Array,
    grad_out: jax.Array,
):
    batch, heads = q.shape[:2]
    bh = batch * heads
    q_spec = pl.BlockSpec((HEADS_PER_STEP, SQ, D), lambda i: (i, 0, 0))
    k_spec = pl.BlockSpec((HEADS_PER_STEP, SK, D), lambda i: (i, 0, 0))
    q_like = jax.ShapeDtypeStruct((bh, SQ, D), q.dtype)
    k_like = jax.ShapeDtypeStruct((bh, SK, D), q.dtype)
    dv, o, dk, dq = pl.pallas_call(
        _kernel,
        grid=(bh // HEADS_PER_STEP,),
        in_specs=[q_spec, k_spec, k_spec, q_spec],
        out_specs=[k_spec, q_spec, k_spec, q_spec],
        out_shape=[k_like, q_like, k_like, q_like],
        scratch_shapes=_scratch_per_head() * HEADS_PER_STEP,
        compiler_params=pltpu.CompilerParams(
            dimension_semantics=("arbitrary",),
            vmem_limit_bytes=100 * 1024 * 1024,
            disable_bounds_checks=True,
        ),
        name="mha_kernel",
    )(q.reshape(bh, SQ, D), k.reshape(bh, SK, D), v.reshape(bh, SK, D), grad_out.reshape(bh, SQ, D))
    return (o.reshape(q.shape), dq.reshape(q.shape), dk.reshape(k.shape), dv.reshape(k.shape))
```

```python
import jax
import jax.numpy as jnp
from jax import lax
import jax.experimental.pallas as pl
import jax.experimental.pallas.tpu as pltpu

NT = (((1,), (1,)), ((), ()))
NN = (((1,), (0,)), ((), ()))
f32 = jnp.float32
bf16 = jnp.bfloat16

SQ, SK, D = 512, 1024, 256
HQ, HK, HD = SQ // 2, SK // 2, D // 2
HEADS_PER_STEP = 2
SCALE = D ** -0.5
EXP2_SCALE = SCALE * 1.4426950408889634

NAMES = ["a", "b", "c", "d", "e", "11", "22"]
LHS_ROLE = ["a", "b", "11", "22", "c", "d", "e"]
RHS_ROLE = ["a", "11", "e", "d", "22", "c", "b"]
TN_ORDER = (2, 4, 3, 5, 1, 6, 7)

LAM = [-1.0, -0.28125, 0.28125, 1.0]
PAIRS = [(0, 1), (2, 3), (0, 2), (1, 3), (0, 3), (1, 2)]
RIDERS = [("u", 1), ("u", 2), ("w", 2), ("u", 3), ("w", 3), ("w", 1)]
HK_OPS = [("u", 0), ("w", 0)] + [o for p, e in zip(PAIRS, RIDERS) for o in (("x",) + p, ("y",) + p, ("z",) + p, e)]
K_OPS = [o for o in HK_OPS if o[0] != "u"]
Q_OPS = [o for o in HK_OPS if o[0] != "w"]
KB, QB = SK // 4, SQ // 4

PHASES = ["SA", "SB", "dPA", "dPB", "dVA", "OA", "dVB", "OB", "dKA", "dQA", "dKB", "dQB"]
BIN = 128
BASE = {
    "S": ([100] * 16, [32] * 16),
    "dP": ([150] * 8 + [135, 150, 200, 200, 200, 200], [64] * 8 + [50] * 6),
    "dV": ([100, 120, 120, 150, 110, 120, 105, 150, 145, 155, 155, 150, 200, 175],
           [72, 76, 76, 80, 85, 60, 45, 45, 32, 32, 32, 32, 30, 30]),
    "O": ([110, 70, 65, 70, 65, 75, 75, 80, 60, 60, 110, 130, 110, 150], [20] + [16] * 7 + [25] * 6),
    "dK": ([140, 260, 290, 140, 170, 310, 310, 200, 220, 330, 350, 310, 320],
           [100, 90, 97, 85, 75, 80, 80, 42, 26, 35, 32, 32, 32]),
    "dQ": ([110, 70, 300, 70, 125, 100, 390, 80, 220, 100, 420, 150, 400],
           [14, 13, 70, 18, 37, 24, 84, 18, 59, 22, 30, 30, 45]),
}
LEAD_IN = [60, 100, 130, 130]
PLAN = dict(
    wv=0.9, pw=5,
    margin=300, lag=256, p_from=4200,
    ds_in=("O", "dQ", "dV"), qk_in=("S", "dV", "dK"),
    ds_parts=[(0.35, (0, 1)), (0.25, (2,)), (0.4, (3,))],
    qk_parts=[(0.55, (0, 1, 2)), (0.45, (3,))],
)


def _dot(a, b, dims):
    return lax.dot_general(a, b, dims, preferred_element_type=f32)


def _combos(x11, x12, x21, x22):
    return [x11 + x22, x21 + x22, x11 + x12, x21 - x11, x12 - x22, x11, x22]


def _combos_t(x11, x12, x21, x22):
    return [x11 + x22, x12 + x22, x11 + x21, x12 - x11, x21 - x22, x11, x22]


def _cat(xs, axis):
    return lax.concatenate(xs, axis)


def _colsum8(x):
    return jnp.sum(x.reshape(x.shape[0] // 8, 8, x.shape[1]), axis=0)


def _out(left, right):
    return _cat([left, right], 1).astype(bf16)


def _acc(acc, key, x):
    acc[key] = x if key not in acc else acc[key] + x


class _Scaled:
    def __init__(self, x):
        self.m = {1.0: x}

    def axpy(self, y, c):
        a = abs(c)
        if a not in self.m:
            self.m[a] = self.m[1.0] * a
        if y is None:
            return self.m[a] if c > 0 else -self.m[a]
        return y + self.m[a] if c > 0 else y - self.m[a]


class _Timeline:
    def __init__(self):
        self.t = 0
        self.start, self.kind, self.valu, self.vst = {}, [], [], []
        for name in PHASES:
            self.start[name] = BIN * len(self.valu)
            valu, vst = BASE[name[:-1]]
            if name[:-1] in ("dV", "dK"):
                for n, x in enumerate(LEAD_IN):
                    self.valu[n - len(LEAD_IN)] += x
                    self.vst[n - len(LEAD_IN)] += x / 6
            self.kind += [name[:-1]] * len(valu)
            self.valu += valu
            self.vst += vst
        self.bins = [[] for _ in self.valu]
        self.groups, self.movable, self.tasks = [], {}, []

    def _put(self, k, group, valu, vst):
        self.valu[k] += valu
        self.vst[k] += vst
        self.bins[k].append((group, valu))

    def spread(self, fns, t0, t1, valu, vst):
        self.groups.append(fns)
        for i in range(len(fns)):
            self._put(int(t0 + (t1 - t0) * i / len(fns)) // BIN, len(self.groups) - 1, valu, vst)

    def fill(self, fns, t0, t1, valu, vst, kinds=None):
        self.groups.append(fns)
        ks = [k for k in range(-(-t0 // BIN), t1 // BIN) if kinds is None or self.kind[k] in kinds]
        self.movable[len(self.groups) - 1] = (ks, vst)
        for _ in fns:
            k = min(ks, key=lambda k: max((self.valu[k] + valu) / 4, PLAN["wv"] * (self.vst[k] + vst)))
            self._put(k, len(self.groups) - 1, valu, vst)

    def _rebalance(self):
        cost = lambda valu, vst: (valu / 400) ** PLAN["pw"] + (PLAN["wv"] * vst / 100) ** PLAN["pw"]
        while True:
            best = None
            for k, items in enumerate(self.bins):
                for g, valu in sorted(set(items)):
                    if g not in self.movable:
                        continue
                    ks, vst = self.movable[g]
                    gain = cost(self.valu[k], self.vst[k]) - cost(self.valu[k] - valu, self.vst[k] - vst)
                    for k2 in ks:
                        d = gain - (cost(self.valu[k2] + valu, self.vst[k2] + vst) - cost(self.valu[k2], self.vst[k2]))
                        if k2 != k and d > 1e-9 and (best is None or d > best[0]):
                            best = (d, k, k2, g, valu, vst)
            if best is None:
                return
            _, k, k2, g, valu, vst = best
            self.bins[k].remove((g, valu))
            self.valu[k] -= valu
            self.vst[k] -= vst
            self._put(k2, g, valu, vst)

    def finish(self):
        self._rebalance()
        times = [[] for _ in self.groups]
        for k, items in enumerate(self.bins):
            by = {}
            for g, valu in items:
                by.setdefault(g, []).append(valu)
            seq = sorted(((n + 0.5) / len(v), g, v[n]) for g, v in by.items() for n in range(len(v)))
            parts = lambda g: [f for f, _ in self.groups[g][0]]
            total, cum, last = sum(valu + 8 * len(parts(g)) for _, g, valu in seq), 0, -8
            for _, g, valu in seq:
                for f in parts(g):
                    last = max(int(cum / total * BIN) // 8 * 8, last + 8)
                    assert last < BIN
                    times[g].append(k * BIN + last)
                    cum += valu * f + 8
        for g, fns in enumerate(self.groups):
            self.tasks += list(zip(sorted(times[g]), [fn for strip in fns for _, fn in strip]))
        self.tasks.sort(key=lambda x: x[0])

    def mxu_pass(self, cycles, result):
        t0 = self.t
        self.t += cycles
        for t, fn in self.tasks:
            if t0 <= t < self.t:
                i = (t - t0) * result.shape[0] // cycles // 8
                fn(lax.slice(result, (8 * i, 0), (8 * i + 8, 128)))


class _Head:
    def __init__(self, h, io, scratch, timeline, zeros, never):
        self.h, self.tl, self.z, self.never = h, timeline, zeros, never
        (self.q_ref, self.k_ref, self.v_ref, self.g_ref,
         self.dv_ref, self.o_ref, self.dk_ref, self.dq_ref) = io
        (s0, s1, self.e_buf, self.dp_buf, self.part_buf, self.p_ops, self.ds_ops,
         self.v4, self.v1, self.k_ops, self.g4, self.g1, self.q_ops) = scratch
        self.s_buf = [s0, s1]
        self.m = [None, None]
        self.l = [None, None]
        self.r = [None, None]
        self.rs = [None, None]
        self.t = [[None, None], [None, None]]
        self.delta = [None, None]

    def after(self, x, tile):
        return lax.select(self.never[x.shape], tile, x)

    def _operand(self, ref, half, four, one, name, r0, r1, zi):
        z = self.z[zi]
        if name == "11":
            return ref[self.h + z, r0:r1, 0:HD]
        if name == "22":
            return ref[self.h + z, half + r0:half + r1, HD:]
        if name == "e":
            return one[z, r0:r1, :]
        c = "abcd".index(name)
        return four[z, r0:r1, c * HD:(c + 1) * HD]

    def v_op(self, name, r0=0, r1=HK, zi=1):
        return self._operand(self.v_ref, HK, self.v4, self.v1, name, r0, r1, zi)

    def g_op(self, name, r0=0, r1=HQ, zi=1):
        return self._operand(self.g_ref, HQ, self.g4, self.g1, name, r0, r1, zi)

    def p_op(self, name, r0, r1, zi):
        c = NAMES.index(name)
        return self.p_ops[self.z[zi], r0:r1, c * HQ:(c + 1) * HQ]

    def k_op(self, o):
        z = self.z[1]
        if o[0] == "u":
            return self.k_ref[self.h + z, o[1] * KB:(o[1] + 1) * KB, 0:HD]
        c = K_OPS.index(o)
        return self.k_ops[z, :, c * HD:(c + 1) * HD]

    def q_op(self, o, zi):
        z = self.z[zi]
        if o[0] == "w":
            return self.q_ref[self.h + z, o[1] * QB:(o[1] + 1) * QB, HD:]
        c = Q_OPS.index(o)
        return self.q_ops[z, :, c * HD:(c + 1) * HD]

    def ds_op(self, o, r0, r1):
        c = HK_OPS.index(o)
        return self.ds_ops[self.z[1], r0:r1, c * 128:(c + 1) * 128]

    def scores(self, j):
        s = _dot(self.k_ref[self.h + self.z[2 + j]], self.q_ref[self.h, j * HQ:(j + 1) * HQ, :], NT)
        sp = s * EXP2_SCALE
        self.s_buf[j][self.z[0]] = sp
        self.m[j] = jnp.broadcast_to(jnp.max(sp, axis=0, keepdims=True), (8, HQ))
        self.tl.mxu_pass(1024, s)

    def _put_dp(self, j, n, row, val):
        cols = slice(n * 128, (n + 1) * 128)
        rows = slice(row, row + val.shape[0])
        self.dp_buf[self.z[0], j, rows, cols] = val
        x = _colsum8(val * self.e_buf[self.z[1], j, rows, cols])
        self.t[j][n] = x if self.t[j][n] is None else self.t[j][n] + x

    def dprobs(self):
        def unit(i, n, r0, r1):
            return _dot(self.v_op(RHS_ROLE[i - 1], r0, r1, 1 + n),
                        self.g_op(LHS_ROLE[i - 1], n * 128, (n + 1) * 128), NT)

        for n in range(2):
            cols = slice(n * 128, (n + 1) * 128)
            m2, m3, m4, m5 = [unit(i, n, 0, HK) for i in (2, 3, 4, 5)]
            self._put_dp(0, n, HK, m3 + m5)
            self._put_dp(1, n, 0, m2 + m4)
            self.part_buf[self.z[0], 0, :, cols] = m4 - m5
            self.part_buf[self.z[0], 1, :, cols] = m3 - m2
            self.tl.mxu_pass(512, m5)
        half = HK // 2
        order = [(i, n, s) for n in range(2) for s in range(2) for i in (1, 6, 7)]
        m, done = {}, set()
        for p in range(3):
            for i, n, s in order[4 * p:4 * p + 4]:
                m[i, n, s] = unit(i, n, s * half, (s + 1) * half)
            for n in range(2):
                for s in range(2):
                    for j, i in ((0, 7), (1, 6)):
                        if (i, n, s) in m and (1, n, s) in m and (i, n, s) not in done:
                            done.add((i, n, s))
                            x = self.part_buf[self.z[1], j, s * half:(s + 1) * half, n * 128:(n + 1) * 128]
                            self._put_dp(j, n, j * HK + s * half, x + m[1, n, s] + m[i, n, s])
            self.tl.mxu_pass(256, m[order[4 * p + 3]])
        for j in range(2):
            t = jnp.sum(_cat(self.t[j], 1), axis=0, keepdims=True)
            self.delta[j] = jnp.broadcast_to(t, (8, HQ)) * self.r[j]
            self.rs[j] = self.r[j] * SCALE

    def dvalues(self):
        self.p_t = {n: self.p_op(n, 0, HK, 2).T for n in [RHS_ROLE[i - 1] for i in TN_ORDER]}

        def prod(i, r0=0, r1=HK):
            return _dot(self.p_op(LHS_ROLE[i - 1], r0, r1, 1),
                        self.g_op(RHS_ROLE[i - 1], zi=(2 if r0 == 0 else 3)), NN)

        m2, m4 = prod(2), prod(4)
        self.tl.mxu_pass(512, m4)
        m3, m5 = prod(3), prod(5)
        self.tl.mxu_pass(512, m5)
        m1, m6 = prod(1), prod(6)
        self.dv_ref[self.h, HK:, :] = _out(m2 + m4, (m3 - m2) + (m1 + m6))
        self.tl.mxu_pass(512, m6)
        m7 = [prod(7, 0, HK // 2), prod(7, HK // 2, HK)]
        self.dv_ref[self.h, 0:HK, :] = _out((m4 - m5) + (m1 + _cat(m7, 0)), m3 + m5)
        self.tl.mxu_pass(256, m7[1])

    def output(self):
        m = {}
        for i in TN_ORDER:
            m[i] = _dot(self.p_t[RHS_ROLE[i - 1]], self.v_op(LHS_ROLE[i - 1], zi=3), NN)
            if i == 6:
                self.o_ref[self.h, HQ:, :] = _out(m[3] + m[5], (m[3] - m[2]) + (m[1] + m[6]))
            if i == 7:
                self.o_ref[self.h, 0:HQ, :] = _out((m[4] - m[5]) + (m[1] + m[7]), m[2] + m[4])
            self.tl.mxu_pass(256, m[i])

    def dkeys(self):
        self.ds_t = [self.ds_ops[self.z[2], :, m * 256:(m + 1) * 256].T for m in range(13)]
        acc = {}

        def prod(o, r0=0, r1=KB, zi=2):
            return _dot(self.ds_op(o, r0, r1), self.q_op(o, zi), NN)

        def single(o, r):
            if o[0] == "u":
                _acc(acc, (o[1], 0), r)
            else:
                acc[o[1], 0] = _Scaled(r).axpy(acc.get((o[1], 0)), -LAM[o[1]])
                _acc(acc, (o[1], 1), r)

        first = [[prod(o, 0, KB // 2), prod(o, KB // 2, KB, 3)] for o in HK_OPS[0:2]]
        for o, r in zip(HK_OPS[0:2], first):
            single(o, _cat(r, 0))
        self.tl.mxu_pass(128, first[1][1])
        left = [3] * 4
        for p, ((i, j), rider) in enumerate(zip(PAIRS, RIDERS)):
            x, y, z, e = [prod(o) for o in HK_OPS[2 + 4 * p:6 + 4 * p]]
            c = x + (y + z)
            sign = 1.0 if LAM[j] > 0 else -1.0
            if LAM[i] == -LAM[j]:
                u = _Scaled(y - z).axpy(None, LAM[j])
            else:
                u = _Scaled(z).axpy(_Scaled(y).axpy(None, sign * LAM[j]), sign * LAM[i])
            single(rider, e)
            sx = _Scaled(x)
            for t in (i, j):
                _acc(acc, (t, 1), c)
                acc[t, 0] = _Scaled(sx.axpy(u, sign * LAM[t])).axpy(acc.get((t, 0)), -sign)
                left[t] -= 1
                if left[t] == 0:
                    self.dk_ref[self.h, t * KB:(t + 1) * KB, :] = _out(acc[t, 0], acc[t, 1])
            self.tl.mxu_pass(256, e)

    def dqueries(self):
        acc = {}

        def prods(m):
            return [_dot(self.ds_t[m][s * QB:(s + 1) * QB], self.k_op(HK_OPS[2 * m + s]), NN) for s in range(2)]

        def single(o, r):
            if o[0] == "u":
                _acc(acc, (o[1], 0), r)
                acc[o[1], 1] = _Scaled(r).axpy(acc.get((o[1], 1)), LAM[o[1]])
            else:
                _acc(acc, (o[1], 1), r)

        first = prods(0)
        for o, r in zip(HK_OPS[0:2], first):
            single(o, r)
        self.tl.mxu_pass(128, first[1])
        left = [3] * 4
        for p, ((i, j), rider) in enumerate(zip(PAIRS, RIDERS)):
            a = 1.0 / (LAM[i] - LAM[j])
            x, y = prods(1 + 2 * p)
            self.tl.mxu_pass(128, y)
            z, e = prods(2 + 2 * p)
            c = (x - (y + z)) * a
            if LAM[i] == -LAM[j]:
                w = (y - z) * (a * LAM[i])
            else:
                w = y * (a * LAM[i]) + z * (a * LAM[j])
            sx = _Scaled(x)
            single(rider, e)
            _acc(acc, (i, 0), c)
            acc[j, 0] = _Scaled(c).axpy(acc.get((j, 0)), -1.0)
            acc[i, 1] = _Scaled(sx.axpy(w, -a * LAM[i])).axpy(acc.get((i, 1)), -1.0)
            _acc(acc, (j, 1), sx.axpy(w, -a * LAM[j]))
            for t in (i, j):
                left[t] -= 1
                if left[t] == 0:
                    self.dq_ref[self.h, t * QB:(t + 1) * QB, :] = _out(acc[t, 0], acc[t, 1])
            self.tl.mxu_pass(128, e)

    def input_combos(self, ref, half, fn, four, one, rows=16):
        def strip(r0):
            def run(tile):
                tile = _cat([tile] * (rows // 8), 0)
                top = ref[self.h, r0:r0 + rows, :].astype(f32)
                bot = ref[self.h, half + r0:half + r0 + rows, :].astype(f32)
                c = fn(self.after(top[:, 0:HD], tile), top[:, HD:], bot[:, 0:HD], self.after(bot[:, HD:], tile))
                four[self.z[0], r0:r0 + rows, :] = _cat(c[0:4], 1).astype(bf16)
                one[self.z[0], r0:r0 + rows, :] = c[4].astype(bf16)
            return [(1.0, run)]
        return [strip(r0) for r0 in range(0, half, rows)]

    def exponentials(self, j, rows):
        def strip(r0):
            def run(tile):
                m = self.after(self.m[j], _cat([tile, tile], 1))
                e = jnp.exp2(self.s_buf[j][self.z[1], r0:r0 + rows, :] - _cat([m] * (rows // 8), 0))
                self.e_buf[self.z[0], j, r0:r0 + rows, :] = e
                e = _colsum8(e)
                self.l[j] = e if self.l[j] is None else self.l[j] + e
                if r0 + rows == SK:
                    l = jnp.sum(self.l[j], axis=0, keepdims=True)
                    self.r[j] = jnp.broadcast_to(1.0 / l, (8, HQ))
            return [(1.0, run)]
        return [strip(r0) for r0 in range(0, SK, rows)]

    def prob_combos(self):
        def strip(r0):
            def run(tile):
                tile = _cat([tile, tile], 1)
                r = [self.after(x, tile) for x in self.r]
                p = [self.e_buf[self.z[1], j, i * HK + r0:i * HK + r0 + 8, :] * r[j] for i in range(2) for j in range(2)]
                self.p_ops[self.z[0], r0:r0 + 8, :] = _cat(_combos(*p), 1).astype(bf16)
            return [(1.0, run)]
        return [strip(r0) for r0 in range(0, HK, 8)]

    def dscore_combos(self):
        def strip(r0):
            ds = {}

            def part(kbs):
                def run(tile):
                    tile = _cat([tile, tile], 1)
                    r = [self.after(x, tile) for x in self.rs]
                    for kb in kbs:
                        rows = slice(kb * KB + r0, kb * KB + r0 + 8)
                        for j in range(2):
                            x = (self.e_buf[self.z[1], j, rows, :] * r[j]) * (self.dp_buf[self.z[1], j, rows, :] - self.delta[j])
                            ds[2 * j, kb], ds[2 * j + 1, kb] = x[:, 0:128], x[:, 128:]
                    if len(ds) < 16:
                        return
                    d = {}
                    for i in range(4):
                        o = [t for t in range(4) if t != i]
                        d["u", i] = (ds[0, i] + ds[1, i]) + (ds[2, i] + ds[3, i])
                        d["w", i] = (ds[i, i] - ds[i, o[0]]) - (ds[i, o[1]] + ds[i, o[2]])
                    for i, j in PAIRS:
                        d["x", i, j], d["y", i, j], d["z", i, j] = ds[i, j] + ds[j, i], ds[j, i], ds[i, j]
                    self.ds_ops[self.z[0], r0:r0 + 8, :] = _cat([d[o] for o in HK_OPS], 1).astype(bf16)
                return run
            return [(f, part(kbs)) for f, kbs in PLAN["ds_parts"]]
        return [strip(r0) for r0 in range(0, KB, 8)]

    def _block_strip(self, ref, block, r0, gate_half, finish):
        x = {}

        def part(blocks):
            def run(tile):
                for i in blocks:
                    y = ref[self.h, i * block + r0:i * block + r0 + 8, :].astype(f32)
                    x[i] = [y[:, 0:HD], y[:, HD:]]
                    x[i][gate_half] = self.after(x[i][gate_half], tile)
                if len(x) == 4:
                    finish([x[i][0] for i in range(4)], [x[i][1] for i in range(4)])
            return run
        return [(f, part(blocks)) for f, blocks in PLAN["qk_parts"]]

    def key_combos(self):
        def strip(r0):
            def finish(k1, k2):
                d = {("w", i): _Scaled(k1[i]).axpy(k2[i], -LAM[i]) for i in range(4)}
                for i, j in PAIRS:
                    s1, s2 = _Scaled(k1[i] + k1[j]), k2[i] + k2[j]
                    d["x", i, j] = d["w", i] + d["w", j]
                    d["y", i, j] = s1.axpy(s2, -LAM[j])
                    d["z", i, j] = s1.axpy(s2, -LAM[i])
                self.k_ops[self.z[0], r0:r0 + 8, :] = _cat([d[o] for o in K_OPS], 1).astype(bf16)
            return self._block_strip(self.k_ref, KB, r0, 0, finish)
        return [strip(r0) for r0 in range(0, KB, 8)]

    def query_combos(self):
        def strip(r0):
            def finish(q1, q2):
                d = {("u", i): _Scaled(q2[i]).axpy(q1[i], LAM[i]) for i in range(4)}
                for i, j in PAIRS:
                    a = 1.0 / (LAM[i] - LAM[j])
                    d1, d2 = (q1[j] - q1[i]) * a, _Scaled(q2[j] - q2[i])
                    d["x", i, j] = (d["u", i] - d["u", j]) * a
                    d["y", i, j] = d2.axpy(d1, a * LAM[i])
                    d["z", i, j] = d2.axpy(d1, a * LAM[j])
                self.q_ops[self.z[0], r0:r0 + 8, :] = _cat([d[o] for o in Q_OPS], 1).astype(bf16)
            return self._block_strip(self.q_ref, QB, r0, 1, finish)
        return [strip(r0) for r0 in range(0, QB, 8)]


def _kernel(*refs):
    io, scratch = refs[:8], refs[8:]
    step = pl.program_id(0)
    zeros = [step >> 12, 0, step >> 14, step >> 15]
    never = {s: jnp.full(s, step >> 16, jnp.int32) != 0 for s in ((8, 256), (16, 128), (8, 128))}
    tl = _Timeline()
    n = len(scratch) // 2
    heads = {"A": _Head(0, io, scratch[:n], tl, zeros, never), "B": _Head(1, io, scratch[n:], tl, zeros, never)}
    a, b = heads["A"], heads["B"]

    at, margin, lag = tl.start, PLAN["margin"], PLAN["lag"]
    assert 3072 + lag <= min(PLAN["p_from"], at["dPA"]) and 5120 + lag <= at["dPB"]
    for i, (x, j) in enumerate(((a, 0), (a, 1), (b, 0), (b, 1))):
        tl.spread(x.exponentials(j, 16), 1024 * (i + 1) + lag, 1024 * (i + 2) + lag, 10.8, 4)
    for h, x in heads.items():
        tl.fill(x.dscore_combos(), at["dP" + h] + 1942, at["dK" + h] - margin, 91 + 4 * len(PLAN["ds_parts"]), 13, PLAN["ds_in"])
    tl.fill(a.prob_combos(), PLAN["p_from"], at["dVA"] - margin, 29, 7)
    for h, x in heads.items():
        tl.fill(x.input_combos(x.g_ref, HQ, _combos, x.g4, x.g1) + x.input_combos(x.v_ref, HK, _combos_t, x.v4, x.v1),
                0, at["dP" + h] - margin, 28, 5.5)
    for h, x in heads.items():
        tl.fill(x.query_combos(), 0, at["dK" + h] - margin, 81, 11, PLAN["qk_in"])
    for h, x in heads.items():
        tl.fill(x.key_combos(), 0, at["dQ" + h] - margin, 62, 11, PLAN["qk_in"])
    tl.fill(b.prob_combos(), at["dVA"], at["dVB"] - margin, 29, 7)
    tl.finish()

    for name in PHASES:
        x = heads[name[-1]]
        if name[:-1] == "S":
            x.scores(0)
            x.scores(1)
        else:
            {"dP": x.dprobs, "dV": x.dvalues, "O": x.output, "dK": x.dkeys, "dQ": x.dqueries}[name[:-1]]()


def _scratch_per_head():
    v = pltpu.VMEM
    return [
        v((1, SK, HQ), f32), v((1, SK, HQ), f32),
        v((1, 2, SK, HQ), f32), v((1, 2, SK, HQ), f32),
        v((1, 2, HK, HQ), f32),
        v((1, HK, 7 * HQ), bf16), v((1, KB, 26 * 128), bf16),
        v((1, HK, 4 * HD), bf16), v((1, HK, HD), bf16),
        v((1, KB, 22 * HD), bf16),
        v((1, HQ, 4 * HD), bf16), v((1, HQ, HD), bf16),
        v((1, QB, 22 * HD), bf16),
    ]


@jax.jit
def pallas_standalone__mha_softmax__near_ridge_kernel(
    q: jax.Array,
    k: jax.Array,
    v: jax.Array,
    grad_out: jax.Array,
):
    batch, heads = q.shape[:2]
    bh = batch * heads
    assert q.shape[2:] == (SQ, D) and k.shape[2:] == (SK, D)
    assert bh % HEADS_PER_STEP == 0 and bh // HEADS_PER_STEP < 4096
    q_spec = pl.BlockSpec((HEADS_PER_STEP, SQ, D), lambda i: (i, 0, 0))
    k_spec = pl.BlockSpec((HEADS_PER_STEP, SK, D), lambda i: (i, 0, 0))
    q_like = jax.ShapeDtypeStruct((bh, SQ, D), q.dtype)
    k_like = jax.ShapeDtypeStruct((bh, SK, D), q.dtype)
    dv, o, dk, dq = pl.pallas_call(
        _kernel,
        grid=(bh // HEADS_PER_STEP,),
        in_specs=[q_spec, k_spec, k_spec, q_spec],
        out_specs=[k_spec, q_spec, k_spec, q_spec],
        out_shape=[k_like, q_like, k_like, q_like],
        scratch_shapes=_scratch_per_head() * HEADS_PER_STEP,
        compiler_params=pltpu.CompilerParams(
            dimension_semantics=("arbitrary",),
            vmem_limit_bytes=100 * 1024 * 1024,
            disable_bounds_checks=True,
        ),
        name="mha_kernel",
    )(q.reshape(bh, SQ, D), k.reshape(bh, SK, D), v.reshape(bh, SK, D), grad_out.reshape(bh, SQ, D))
    return (o.reshape(q.shape), dq.reshape(q.shape), dk.reshape(k.shape), dv.reshape(k.shape))
```
